```python
import jax
import jax.numpy as jnp

def _softmax(x, axis=-1):
    return jax.nn.softmax(x, axis=axis)
def _gelu(x):
    return jax.nn.gelu(x, approximate=True)
def _silu(x):
    return jax.nn.silu(x)
def _sigmoid(x):
    return jax.nn.sigmoid(x)
def _layernorm(x, axis=-1, eps=1e-5):
    m = jnp.mean(x, axis=axis, keepdims=True)
    v = jnp.var(x, axis=axis, keepdims=True)
    return (x - m) / jnp.sqrt(v + eps)
def _scatter_add(tgt, idx, src, axis=0):
    return tgt.at[idx].add(src)
def _segment_sum(src, seg, n):
    return jax.ops.segment_sum(src, seg, n)
class _Rng:
    def __init__(self, key):
        self._k = key
    def _next(self):
        self._k, sub = jax.random.split(self._k)
        return sub
    def normal(self, shape):
        return jax.random.normal(self._next(), shape, dtype=jnp.bfloat16)
    def randint(self, lo, hi, shape):
        return jax.random.randint(self._next(), shape, lo, hi, dtype=jnp.int32)
    def uniform(self, shape, lo=0.0, hi=1.0):
        return jax.random.uniform(self._next(), shape, jnp.bfloat16, lo, hi)
    def permutation(self, n):
        return jax.random.permutation(self._next(), n)


kernel_name = 'standalone__dcn_v2_cross__recsys'

def setup_inputs():
    _rng = _Rng(jax.random.key(int.from_bytes(__import__("os").urandom(4), "little")))
    _w = (lambda a: (lambda t: t.astype(jnp.bfloat16) if jnp.issubdtype(t.dtype, jnp.floating) else t)(jnp.asarray(a)))
    B, F, D, L = 16384, 26, 128, 6
    Din = min(F * D, 1024)
    return {
        "x0": _w((lambda *s: _rng.normal(s) * 0.05)(B, Din)),
        "ws": _w((lambda *s: _rng.normal(s) * 0.05)(L, Din, Din)),
        "bs": _w((lambda *s: _rng.normal(s) * 0.05)(L, Din)),
    }

def reference(x0, ws, bs):
    x = x0
    for l in range(ws.shape[0]):
        x = x0 * (x @ ws[l] + bs[l]) + x
    return x
```

```python
import jax
import jax.numpy as jnp
import jax.experimental.pallas as pl
import jax.experimental.pallas.tpu as pltpu

_BM = 512
_SUB = 256


def _kernel(x0_ref, w_ref, b_ref, o_ref):
    n_layers = w_ref.shape[0]
    for s in range(_BM // _SUB):
        rows = pl.ds(s * _SUB, _SUB)
        xb = x0_ref[rows, :]
        x0f = xb.astype(jnp.float32)
        x = x0f
        for l in range(n_layers):
            y = jnp.dot(xb, w_ref[l], preferred_element_type=jnp.float32)
            x = x0f * (y + b_ref[l:l + 1, :].astype(jnp.float32)) + x
            xb = x.astype(jnp.bfloat16)
        o_ref[rows, :] = xb


@jax.jit
def pallas_standalone__dcn_v2_cross__recsys_kernel(
    x0: jax.Array,
    ws: jax.Array,
    bs: jax.Array,
):
    B, D = x0.shape
    return pl.pallas_call(
        _kernel,
        grid=(B // _BM,),
        in_specs=[
            pl.BlockSpec((_BM, D), lambda i: (i, 0)),
            pl.BlockSpec(ws.shape, lambda i: (0, 0, 0), pipeline_mode=pl.Buffered(1)),
            pl.BlockSpec(bs.shape, lambda i: (0, 0), pipeline_mode=pl.Buffered(1)),
        ],
        out_specs=pl.BlockSpec((_BM, D), lambda i: (i, 0)),
        out_shape=jax.ShapeDtypeStruct(x0.shape, x0.dtype),
        compiler_params=pltpu.CompilerParams(
            dimension_semantics=("arbitrary",),
            vmem_limit_bytes=100 * 1024 * 1024,
        ),
    )(x0, ws, bs)
```

```python
import jax
import jax.numpy as jnp
from jax import lax
import jax.experimental.pallas as pl
import jax.experimental.pallas.tpu as pltpu

_BM = 512
_SUB = 256


def _layer(x0, xb, w, b):
    y = jnp.dot(xb, w, preferred_element_type=jnp.float32)
    x = x0.astype(jnp.float32) * (y + b) + xb.astype(jnp.float32)
    return x.astype(jnp.bfloat16)


def _kernel(x0_hbm, w_hbm, b_hbm, o_hbm,
            w_v, b_v, bf, xin, obuf, wsem, bsem, xsem, osem):
    n = x0_hbm.shape[0] // _BM
    L = w_hbm.shape[0]

    def w_cp(l):
        return pltpu.make_async_copy(w_hbm.at[l], w_v.at[l], wsem.at[l])

    def x_cp(t, s):
        return pltpu.make_async_copy(
            x0_hbm.at[pl.ds(t * _BM, _BM)], xin.at[s], xsem.at[s])

    def o_cp(t, s):
        return pltpu.make_async_copy(
            obuf.at[s], o_hbm.at[pl.ds(t * _BM, _BM)], osem.at[s])

    b_cp = pltpu.make_async_copy(b_hbm, b_v, bsem.at[0])

    b_cp.start()
    x_cp(0, 0).start()
    w_cp(0).start()
    b_cp.wait()
    for l in range(L):
        bf[l] = b_v[l:l + 1, :].astype(jnp.float32)
    x_cp(0, 0).wait()
    obuf[0] = xin[0]

    def first(l, c):
        w_cp(l).wait()

        @pl.when(l + 1 < L)
        def _():
            w_cp(l + 1).start()

        @pl.when(l == L - 1)
        def _():
            x_cp(1, 1).start()

        for s in range(_BM // _SUB):
            rows = pl.ds(s * _SUB, _SUB)
            obuf[0, rows, :] = _layer(
                xin[0, rows, :], obuf[0, rows, :], w_v[l], bf[l])
        return c

    lax.fori_loop(0, L, first, 0)
    o_cp(0, 0).start()

    def body(t, c):
        slot = lax.rem(t, 2)

        @pl.when(t + 1 < n)
        def _():
            x_cp(t + 1, 1 - slot).start()

        x_cp(t, slot).wait()

        @pl.when(t >= 2)
        def _():
            o_cp(t - 2, slot).wait()

        for s in range(_BM // _SUB):
            rows = pl.ds(s * _SUB, _SUB)
            xb = xin[slot, rows, :]
            for l in range(L):
                xb = _layer(xin[slot, rows, :], xb, w_v[l], bf[l])
            obuf[slot, rows, :] = xb
        o_cp(t, slot).start()
        return c

    lax.fori_loop(1, n, body, 0)
    o_cp(n - 2, n % 2).wait()
    o_cp(n - 1, (n - 1) % 2).wait()


@jax.jit
def pallas_standalone__dcn_v2_cross__recsys_kernel(
    x0: jax.Array,
    ws: jax.Array,
    bs: jax.Array,
):
    B, D = x0.shape
    L = ws.shape[0]
    assert B % _BM == 0 and B // _BM >= 2
    hbm = pl.BlockSpec(memory_space=pl.ANY)
    return pl.pallas_call(
        _kernel,
        in_specs=[hbm, hbm, hbm],
        out_specs=hbm,
        out_shape=jax.ShapeDtypeStruct(x0.shape, x0.dtype),
        scratch_shapes=[
            pltpu.VMEM(ws.shape, ws.dtype),
            pltpu.VMEM(bs.shape, bs.dtype),
            pltpu.VMEM((L, 1, D), jnp.float32),
            pltpu.VMEM((2, _BM, D), x0.dtype),
            pltpu.VMEM((2, _BM, D), x0.dtype),
            pltpu.SemaphoreType.DMA((L,)),
            pltpu.SemaphoreType.DMA((1,)),
            pltpu.SemaphoreType.DMA((2,)),
            pltpu.SemaphoreType.DMA((2,)),
        ],
        compiler_params=pltpu.CompilerParams(vmem_limit_bytes=64 * 1024 * 1024),
    )(x0, ws, bs)
```
